```python
import os as _os
_os.environ.setdefault("JAX_PLATFORMS", "cpu")
import jax
import jax.numpy as jnp

def _softmax(x, axis=-1):
    return jax.nn.softmax(x, axis=axis)
def _gelu(x):
    return jax.nn.gelu(x, approximate=True)
def _silu(x):
    return jax.nn.silu(x)
def _sigmoid(x):
    return jax.nn.sigmoid(x)
def _layernorm(x, axis=-1, eps=1e-5):
    m = jnp.mean(x, axis=axis, keepdims=True)
    v = jnp.var(x, axis=axis, keepdims=True)
    return (x - m) / jnp.sqrt(v + eps)
def _scatter_add(tgt, idx, src, axis=0):
    return tgt.at[idx].add(src)
def _segment_sum(src, seg, n):
    return jax.ops.segment_sum(src, seg, n)
class _Rng:
    def __init__(self, key):
        self._k = key
    def _next(self):
        self._k, sub = jax.random.split(self._k)
        return sub
    def normal(self, shape):
        return jax.random.normal(self._next(), shape, dtype=jnp.bfloat16)
    def randint(self, lo, hi, shape):
        return jax.random.randint(self._next(), shape, lo, hi, dtype=jnp.int32)
    def uniform(self, shape, lo=0.0, hi=1.0):
        return jax.random.uniform(self._next(), shape, jnp.bfloat16, lo, hi)
    def permutation(self, n):
        return jax.random.permutation(self._next(), n)


kernel_name = 'gated_mix__compressed_kv_cla__linear_attn_block__prompt'

def setup_inputs():
    _rng = _Rng(jax.random.key(int.from_bytes(__import__("os").urandom(4), "little")))
    _w = (lambda a: (lambda t: t.astype(jnp.bfloat16) if jnp.issubdtype(t.dtype, jnp.floating) else t)(jnp.asarray(a)))
    def _A_setup():
        B, H, Sq, Sk, D, M = 1, 16, 2048, 2048, 256, 448
        Dc = 4 * D
        return {
            "x": _w((lambda *s: _rng.normal(s) * 0.05)(B, Sq, M)),
            "c_kv": _w((lambda *s: _rng.normal(s) * 0.8)(B, Sk, Dc)),
            "w_q": _w((lambda *s: _rng.normal(s) * 3.2)(M, H, D) * (M ** -0.5)),
            "w_uk": _w((lambda *s: _rng.normal(s) * 3.2)(Dc, H, D) * (Dc ** -0.5)),
            "w_uv": _w((lambda *s: _rng.normal(s) * 0.8)(Dc, H, D) * (Dc ** -0.5)),
            "w_o": _w((lambda *s: _rng.normal(s) * 0.8)(H, D, M) * ((H * D) ** -0.5)),
        }
    _A_in = _A_setup()

    def _B_setup():
        B, S, D = 1, 2048, 448
        return {
            "x": _w((lambda *s: _rng.normal(s) * 0.05)(B, S, D)),
            "wqkv": _w((lambda *s: _rng.normal(s) * 1.6)(D, 3 * D)),
            "wo": _w((lambda *s: _rng.normal(s) * 0.4)(D, D)),
        }
    _B_in = _B_setup()

    return {
        "A_x": _A_in["x"],
        "A_c_kv": _A_in["c_kv"],
        "A_w_q": _A_in["w_q"],
        "A_w_uk": _A_in["w_uk"],
        "A_w_uv": _A_in["w_uv"],
        "A_w_o": _A_in["w_o"],
        "B_x": _B_in["x"],
        "B_wqkv": _B_in["wqkv"],
        "B_wo": _B_in["wo"],
        "gate_w": _w((lambda *s: _rng.normal(s) * 0.05)(448) * 16.0),
    }

def reference(A_x, A_c_kv, A_w_q, A_w_uk, A_w_uv, A_w_o, B_x, B_wqkv, B_wo, gate_w):
    def _A_ref(x, c_kv, w_q, w_uk, w_uv, w_o):
        B, Sq, M = x.shape[0], x.shape[1], x.shape[2]
        Sk = c_kv.shape[1]
        H, D = w_q.shape[1], w_q.shape[2]
        q = jnp.einsum("bqm,mhd->bhqd", x, w_q)
        k = jnp.einsum("bkc,chd->bhkd", c_kv, w_uk)
        v = jnp.einsum("bkc,chd->bhkd", c_kv, w_uv)
        scores = jnp.einsum("bhqd,bhkd->bhqk", q, k) * (D ** -0.5)
        off = Sk - Sq
        qi = jnp.arange(Sq)[:, None]
        kj = jnp.arange(Sk)[None, :]
        cmask = kj <= (qi + off)
        scores = jnp.where(cmask[None, None], scores, -1e9)
        p = _softmax(scores, axis=-1)
        ctx = jnp.einsum("bhqk,bhkd->bhqd", p, v)
        return jnp.einsum("bhqd,hdm->bqm", ctx, w_o)

    def _B_ref(x, wqkv, wo):
        B, S, D = x.shape
        H = 16; Dh = D // H
        qkv = (lambda x, *d: x.transpose(*d))((x @ wqkv).reshape(B, S, 3, H, Dh), 2, 0, 3, 1, 4)
        q, k, v = qkv[0], qkv[1], qkv[2]
        phi = lambda t: jnp.where(t > 0, t + 1, jnp.exp(t)) + 1e-6
        pq, pk = phi(q), phi(k)
        kv = jnp.einsum("bhsd,bhse->bhde", pk, v)
        z = jnp.einsum("bhsd->bhd", pk)
        num = jnp.einsum("bhqd,bhde->bhqe", pq, kv)
        den = jnp.einsum("bhqd,bhd->bhq", pq, z)[..., None] + 1e-6
        o = num / den
        return (lambda x, *d: x.transpose(*d))(o, 0, 2, 1, 3).reshape(B, S, D) @ wo

    x = A_x
    g = _sigmoid((x * gate_w).sum(-1, keepdims=True))
    a = _A_ref(x, A_c_kv, A_w_q, A_w_uk, A_w_uv, A_w_o)
    b = _B_ref(x, B_wqkv, B_wo)
    return g * a + (1 - g) * b
```

```python
import functools, math
import numpy as np
import jax, jax.numpy as jnp
from jax import lax
from jax.experimental import pallas as pl
from jax.experimental.pallas import tpu as pltpu

S, M, DC, H, D = 2048, 448, 1024, 16, 256
HB, DH = 16, 28
LOG2E = 1.4426950408889634
NEG = -1e30
BF = jnp.bfloat16
F32 = jnp.float32
U32 = jnp.uint32
T128 = 128

def _nt(a, b):
    return lax.dot_general(a, b, (((1,), (1,)), ((), ())), preferred_element_type=F32)
def _tn(a, b):
    return lax.dot_general(a, b, (((0,), (0,)), ((), ())), preferred_element_type=F32)
def _nn(a, b):
    return jnp.dot(a, b, preferred_element_type=F32)

def ld(ref, r0, r1, c0=None, c1=None):
    cols = slice(None) if c0 is None else slice(c0, c1)
    return pltpu.bitcast(ref[r0 // 2:r1 // 2, cols], BF)
def st(ref, r0, r1, val, c0=None, c1=None):
    cols = slice(None) if c0 is None else slice(c0, c1)
    ref[r0 // 2:r1 // 2, cols] = pltpu.bitcast(val, U32)

def _extract(w_refs, rows, h):
    j = h // 2
    sh = ((h % 2) * 16).astype(U32)
    return [pltpu.bitcast((w[pl.ds(j, rows, stride=8), :] >> sh).astype(jnp.uint16), BF) for w in w_refs]

def kernel(xT_hbm, c_hbm, wq_hbm, wuk_hbm, wuv_hbm, woT_hbm, wqkv_hbm, wob_hbm, gw_hbm,
           o_hbm,
           xT_v, c_v, wq_v0, wq_v1, wuk_v0, wuk_v1, wuv_v0, wuv_v1, woT_v, wqkv_v, wob_v, gw_v, sems, osems,
           acc, b_s, g_s, q_s, k_s, v_s, wq_s, wuk_s, wuv_s, pq_s, pk_s, x_s, o_s, *, BQ, PB, RB, EXT_AT, SCOPES, UNROLL):
    NR = S // RB
    cur = [None]
    class _N:
        def __enter__(self): pass
    def SC(name):
        if SCOPES:
            cur[0] = jax.named_scope(name)
            return cur[0]
        return _N()
    def NX(name):
        if SCOPES:
            cur[0].__exit__(None, None, None)
            if name:
                cur[0] = jax.named_scope(name); cur[0].__enter__()
    xT_b = xT_v.bitcast(BF)
    def cp(src, dst, i):
        return pltpu.make_async_copy(src, dst, sems.at[i])
    c_wqkv = cp(wqkv_hbm, wqkv_v.bitcast(BF), 0)
    c_x = [cp(xT_hbm.at[:, r * RB:(r + 1) * RB], xT_b.at[0:M, r * RB:(r + 1) * RB], 1 + r) for r in range(NR)]
    c_wob = cp(wob_hbm, wob_v.bitcast(BF), 5)
    c_gw = cp(gw_hbm, gw_v, 6)
    c_wq = [cp(wq_hbm.at[:, 0:128], wq_v0.bitcast(BF), 7), cp(wq_hbm.at[:, 128:256], wq_v1.bitcast(BF), 8)]
    c_c = cp(c_hbm, c_v.bitcast(BF), 9)
    c_wuk = [cp(wuk_hbm.at[:, 0:128], wuk_v0.bitcast(BF), 10), cp(wuk_hbm.at[:, 128:256], wuk_v1.bitcast(BF), 11)]
    c_wuv = [cp(wuv_hbm.at[:, 0:128], wuv_v0.bitcast(BF), 12), cp(wuv_hbm.at[:, 128:256], wuv_v1.bitcast(BF), 13)]
    c_wo = cp(woT_hbm, woT_v.bitcast(BF), 14)

    SC("s0_dma0").__enter__()
    c_wqkv.start()
    for c_ in c_x:
        c_.start()
    c_wob.start(); c_gw.start()
    c_wqkv.wait()
    NX("s1_b1")

    def phi(t):
        return jnp.where(t > 0, t + 1.0, jnp.exp(t)) + 1e-6
    wqkT = ld(wqkv_v, 0, M, 0, 2 * M).astype(F32).T.astype(BF)
    wv_b = ld(wqkv_v, 0, M, 2 * M, 3 * M)
    acc[...] = jnp.zeros_like(acc)
    xT_v[M // 2:M // 2 + 8, :] = jnp.full((8, S), 0x3F803F80, U32)
    for r in range(NR):
        c0, c1 = r * RB, (r + 1) * RB
        c_x[r].wait()
        if r == NR - 1:
            c_wq[0].start(); c_wq[1].start(); c_c.start()
            c_wuk[0].start(); c_wuk[1].start()
            c_wuv[0].start(); c_wuv[1].start(); c_wo.start()
        xr = ld(xT_v, 0, M, c0, c1)
        p = phi(_nn(wqkT, xr)).astype(BF)
        st(pq_s, 0, M, p[:M], c0, c1)
        st(pk_s, 0, M, p[M:], c0, c1)
        st(x_s, c0, c1, xr.astype(F32).T.astype(BF))
    NX("s2_gt")
    c_wob.wait(); c_gw.wait()
    GT = _nt(ld(xT_v, 0, M + 16), ld(pk_s, 0, M))
    kvT = _tn(wv_b, GT[:M].astype(BF))
    ri = lax.broadcasted_iota(jnp.int32, (M, M), 0) // DH
    ci = lax.broadcasted_iota(jnp.int32, (M, M), 1) // DH
    kvT = jnp.where(ri == ci, kvT, 0.0).astype(BF)
    TT = _tn(ld(wob_v, 0, M), kvT).astype(BF)
    z = GT[M:M + 1, :]
    rz = lax.broadcasted_iota(jnp.int32, (32, M), 0)
    cz = lax.broadcasted_iota(jnp.int32, (32, M), 1) // DH
    ZcT = jnp.where(rz % HB == cz, z, 0.0).astype(BF)
    re = lax.broadcasted_iota(jnp.int32, (M, 32), 0) // DH
    ce = lax.broadcasted_iota(jnp.int32, (M, 32), 1)
    ET = jnp.where(ce % HB == re, 1.0, 0.0).astype(BF)

    gw8 = jnp.broadcast_to(gw_v[...], (8, M))
    g_s[...] = jax.nn.sigmoid(_nn(gw8, ld(xT_v, 0, M)))

    def b_stage2(r):
        c0, c1 = r * RB, (r + 1) * RB
        pq = ld(pq_s, 0, M, c0, c1)
        den = _nn(ZcT, pq) + 1e-6
        rc = 1.0 / den
        hi = rc.astype(BF)
        lo = (rc - hi.astype(F32)).astype(BF)
        rw = lax.broadcasted_iota(jnp.int32, (32, RB), 0)
        rr = jnp.where(rw < HB, hi, lo)
        rf = _nn(ET, rr)
        o = (pq.astype(F32) * rf).astype(BF)
        b_s[:, c0:c1] = _nn(TT, o)

    NQ = S // BQ
    nsub = BQ // T128

    def extract_one(refs, rows, dst, h):
        hv = _extract(refs, rows, h)
        for half in range(2):
            st(dst, 0, rows, hv[half], half * 128, half * 128 + 128)

    def extract(h):
        extract_one((wuk_v0, wuk_v1), DC, wuk_s, h)
        extract_one((wuv_v0, wuv_v1), DC, wuv_s, h)

    def extract_q_all():
        for j in range(H // 2):
            for half, w in enumerate((wq_v0, wq_v1)):
                a = w[pl.ds(j, M, stride=8), :]
                cols = slice(half * 128, half * 128 + 128)
                wq_s[2 * j, :, cols] = pltpu.bitcast(a.astype(jnp.uint16), U32)
                wq_s[2 * j + 1, :, cols] = pltpu.bitcast((a >> 16).astype(jnp.uint16), U32)

    def q_head(h, carry):
        w = pltpu.bitcast(wq_s[h], BF)
        for r in range(S // PB):
            r0, r1 = r * PB, (r + 1) * PB
            q = (_nn(ld(x_s, r0, r1), w) * (LOG2E / 16.0)).astype(BF)
            q_s[h, r0 // 2:r1 // 2, :] = pltpu.bitcast(q, U32)
        return carry
    def proj_k(r0, r1):
        st(k_s, r0, r1, _nn(ld(c_v, r0, r1), ld(wuk_s, 0, DC)).astype(BF))
    def proj_v(r0, r1):
        st(v_s, r0, r1, _nn(ld(c_v, r0, r1), ld(wuv_s, 0, DC)).astype(BF))
    def proj():
        for r in range(S // PB):
            r0, r1 = r * PB, (r + 1) * PB
            proj_k(r0, r1); proj_v(r0, r1)

    def qk(h, i):
        r0 = i * BQ
        a = lax.broadcasted_iota(jnp.int32, (T128, T128), 0)
        b = lax.broadcasted_iota(jnp.int32, (T128, T128), 1)
        s_diag = []
        q = pltpu.bitcast(q_s[h, r0 // 2:(r0 + BQ) // 2, :], BF)
        for t in range(nsub):
            s = _nt(q[t * T128:(t + 1) * T128, :], ld(k_s, r0, r0 + (t + 1) * T128))
            last = jnp.where(b <= a, s[:, t * T128:], NEG)
            s_diag.append(jnp.concatenate([s[:, :t * T128], last], axis=1) if t > 0 else last)
        m = jnp.concatenate([jnp.max(s, axis=-1, keepdims=True) for s in s_diag], axis=0)
        s_off = None
        if i > 0:
            s_off = _nt(q, ld(k_s, 0, r0))
            m = jnp.maximum(jnp.max(s_off, axis=-1, keepdims=True), m)
        return s_diag, s_off, m

    def pv(i, state):
        s_diag, s_off, m = state
        r0 = i * BQ
        cs, ls = [], []
        for t in range(nsub):
            p = jnp.exp2(s_diag[t] - m[t * T128:(t + 1) * T128, :])
            ls.append(jnp.sum(p, axis=1, keepdims=True))
            cs.append(_nn(p.astype(BF), ld(v_s, r0, r0 + (t + 1) * T128)))
        l = jnp.concatenate(ls, axis=0)
        ctx = jnp.concatenate(cs, axis=0)
        if i > 0:
            p_off = jnp.exp2(s_off - m)
            l = l + jnp.sum(p_off, axis=1, keepdims=True)
            ctx = ctx + _nn(p_off.astype(BF), ld(v_s, 0, r0))
        return (ctx / l).astype(BF)

    def out_copy(i):
        r0 = i * BQ
        return pltpu.make_async_copy(o_s.bitcast(BF).at[:, r0:r0 + BQ], o_hbm.at[:, r0:r0 + BQ], osems.at[i])

    def oproj(i, cn, woT_h, final):
        r0 = i * BQ
        a = acc[:, r0:r0 + BQ] + _nt(woT_h, cn)
        if not final:
            acc[:, r0:r0 + BQ] = a
        else:
            g = g_s[0:1, r0:r0 + BQ]
            st(o_s, 0, M, (g * a + (1.0 - g) * b_s[:, r0:r0 + BQ]).astype(BF), r0, r0 + BQ)
            out_copy(i).start()

    def attention(h, final):
        woT_h = pltpu.bitcast(woT_v[pl.ds(pl.multiple_of(h * (M // 2), M // 2), M // 2), :], BF)
        order = list(range(NQ))[::-1]
        st_ = qk(h, order[0])
        prev = None
        for n, i in enumerate(order):
            nxt = qk(h, order[n + 1]) if n + 1 < NQ else None
            cn = pv(i, st_)
            if prev is not None:
                oproj(order[n - 1], prev, woT_h, final)
            prev = cn
            st_ = nxt
            if n == max(EXT_AT, 0) and EXT_AT != -1 and not final:
                extract(h + 1)
        oproj(order[-1], prev, woT_h, final)

    zero = jnp.int32(0)
    NX("s3_wqwait")
    c_wq[0].wait(); c_wq[1].wait()
    NX("s4_b2")
    extract_q_all()
    for r in range(NR):
        b_stage2(r)
    NX("s5_qloop")
    lax.fori_loop(0, H, q_head, 0)
    NX("s6_wait")
    c_c.wait(); c_wuk[0].wait(); c_wuk[1].wait()
    c_wuv[0].wait(); c_wuv[1].wait(); c_wo.wait()
    NX("s7_proj0")
    extract(zero)
    proj()
    NX("s8_main")

    def head(h, carry):
        if SCOPES == 2:
            with jax.named_scope("l_att"):
                attention(h, False)
            with jax.named_scope("l_proj"):
                proj()
        else:
            attention(h, False)
            proj()
        return carry
    if UNROLL == 15:
        for h in range(H - 1):
            head(jnp.int32(h), 0)
    else:
        def heads(it, carry):
            for j in range(UNROLL):
                head(it * UNROLL + j if EXT_AT != -2 else jnp.int32(3), 0)
            return carry
        lax.fori_loop(0, (H - 1) // UNROLL, heads, 0)
    NX("s9_last")
    attention(jnp.int32(H - 1), True)
    NX("s10_outwait")
    for i in range(NQ):
        out_copy(i).wait()
    NX(None)

def make(BQ=256, PB=512, RB=512, EXT_AT=0, SCOPES=False, UNROLL=1):
    def fn(A_x, A_c_kv, A_w_q, A_w_uk, A_w_uv, A_w_o, B_x, B_wqkv, B_wo, gate_w):
        ins = [A_x.transpose(0, 2, 1).reshape(M, S), A_c_kv.reshape(S, DC), A_w_q.reshape(M * H, D),
               A_w_uk.reshape(DC * H, D), A_w_uv.reshape(DC * H, D),
               A_w_o.transpose(0, 2, 1).reshape(H * M, D), B_wqkv, B_wo,
               gate_w.reshape(1, M)]
        V = pltpu.VMEM
        scratch = [V((M // 2 + 8, S), U32), V((S // 2, DC), U32),
                   V((M * 8, 128), U32), V((M * 8, 128), U32), V((DC * 8, 128), U32), V((DC * 8, 128), U32),
                   V((DC * 8, 128), U32), V((DC * 8, 128), U32),
                   V((H * M // 2, D), U32), V((M // 2, 3 * M), U32), V((M // 2, M), U32), V((1, M), BF)]
        qkv = [V((H, S // 2, D), U32), V((S // 2, D), U32), V((S // 2, D), U32),
               V((H, M // 2, D), U32), V((DC // 2, D), U32), V((DC // 2, D), U32)]
        scratch += [pltpu.SemaphoreType.DMA((15,)), pltpu.SemaphoreType.DMA((S // BQ,)),
                    V((M, S), F32), V((M, S), F32), V((8, S), F32),
                    *qkv,
                    V((M // 2, S), U32), V((M // 2, S), U32), V((S // 2, M), U32), V((M // 2, S), U32)]
        def kern(*refs):
            return kernel(*refs, BQ=BQ, PB=PB, RB=RB, EXT_AT=EXT_AT, SCOPES=SCOPES, UNROLL=UNROLL)
        out = pl.pallas_call(
            kern,
            out_shape=jax.ShapeDtypeStruct((M, S), BF),
            in_specs=[pl.BlockSpec(memory_space=pltpu.HBM)] * 9,
            out_specs=pl.BlockSpec(memory_space=pltpu.HBM),
            scratch_shapes=scratch,
            compiler_params=pltpu.CompilerParams(vmem_limit_bytes=110 * 1024 * 1024),
        )(*ins)
        return out.reshape(1, M, S).transpose(0, 2, 1)
    return fn


_impl = make(UNROLL=15)


@jax.jit
def pallas_gated_mix__compressed_kv_cla__linear_attn_block__prompt_kernel(
    A_x, A_c_kv, A_w_q, A_w_uk, A_w_uv, A_w_o, B_x, B_wqkv, B_wo, gate_w,
):
    return _impl(A_x, A_c_kv, A_w_q, A_w_uk, A_w_uv, A_w_o, B_x, B_wqkv, B_wo, gate_w)
```

```python
import functools, math
import numpy as np
import jax, jax.numpy as jnp
from jax import lax
from jax.experimental import pallas as pl
from jax.experimental.pallas import tpu as pltpu

S, M, DC, H, D = 2048, 448, 1024, 16, 256
HB, DH = 16, 28
LOG2E = 1.4426950408889634
NEG = -1e30
BF = jnp.bfloat16
F32 = jnp.float32
U32 = jnp.uint32
T128 = 128

def _nt(a, b):
    return lax.dot_general(a, b, (((1,), (1,)), ((), ())), preferred_element_type=F32)
def _tn(a, b):
    return lax.dot_general(a, b, (((0,), (0,)), ((), ())), preferred_element_type=F32)
def _nn(a, b):
    return jnp.dot(a, b, preferred_element_type=F32)

def ld(ref, r0, r1, c0=None, c1=None):
    cols = slice(None) if c0 is None else slice(c0, c1)
    return pltpu.bitcast(ref[r0 // 2:r1 // 2, cols], BF)
def st(ref, r0, r1, val, c0=None, c1=None):
    cols = slice(None) if c0 is None else slice(c0, c1)
    ref[r0 // 2:r1 // 2, cols] = pltpu.bitcast(val, U32)

def _extract(w_refs, rows, h):
    j = h // 2
    sh = ((h % 2) * 16).astype(U32)
    return [pltpu.bitcast((w[pl.ds(j, rows, stride=8), :] >> sh).astype(jnp.uint16), BF) for w in w_refs]

def kernel(xT_hbm, c_hbm, wq_hbm, wuk_hbm, wuv_hbm, woT_hbm, wqkv_hbm, wob_hbm, gw_hbm,
           o_hbm,
           xT_v, c_v, wq_v0, wq_v1, wuk_v0, wuk_v1, wuv_v0, wuv_v1, woT_v, wqkv_v, wob_v, gw_v, sems, osems,
           acc, b_s, g_s, q_s, k_s, v_s, wq_s, wuk_s, wuv_s, pq_s, pk_s, x_s, o_s, *, BQ, PB, RB, EXT_AT, SCOPES, UNROLL, QUN, PVC, RCP, ORD):
    NR = S // RB
    cur = [None]
    class _N:
        def __enter__(self): pass
    def SC(name):
        if SCOPES:
            cur[0] = jax.named_scope(name)
            return cur[0]
        return _N()
    def NX(name):
        if SCOPES:
            cur[0].__exit__(None, None, None)
            if name:
                cur[0] = jax.named_scope(name); cur[0].__enter__()
    xT_b = xT_v.bitcast(BF)
    def cp(src, dst, i):
        return pltpu.make_async_copy(src, dst, sems.at[i])
    c_wqkv = cp(wqkv_hbm, wqkv_v.bitcast(BF), 0)
    c_x = [cp(xT_hbm.at[:, r * RB:(r + 1) * RB], xT_b.at[0:M, r * RB:(r + 1) * RB], 1 + r) for r in range(NR)]
    c_wob = cp(wob_hbm, wob_v.bitcast(BF), 5)
    c_gw = cp(gw_hbm, gw_v, 6)
    c_wq = [cp(wq_hbm.at[:, 0:128], wq_v0.bitcast(BF), 7), cp(wq_hbm.at[:, 128:256], wq_v1.bitcast(BF), 8)]
    c_c = cp(c_hbm, c_v.bitcast(BF), 9)
    c_wuk = [cp(wuk_hbm.at[:, 0:128], wuk_v0.bitcast(BF), 10), cp(wuk_hbm.at[:, 128:256], wuk_v1.bitcast(BF), 11)]
    c_wuv = [cp(wuv_hbm.at[:, 0:128], wuv_v0.bitcast(BF), 12), cp(wuv_hbm.at[:, 128:256], wuv_v1.bitcast(BF), 13)]
    c_wo = cp(woT_hbm, woT_v.bitcast(BF), 14)

    SC("s0_dma0").__enter__()
    c_gw.start()
    c_wqkv.start()
    for c_ in c_x:
        c_.start()
    c_wob.start()
    c_wqkv.wait(); c_gw.wait()
    NX("s1_b1")

    def phi(t):
        return jnp.where(t > 0, t + 1.0, jnp.exp(t)) + 1e-6
    gw16 = jnp.broadcast_to(gw_v[...].reshape(1, M), (16, M))
    wqkT = jnp.concatenate([ld(wqkv_v, 0, M, 0, 2 * M).astype(F32).T.astype(BF), gw16], axis=0)
    wv_b = ld(wqkv_v, 0, M, 2 * M, 3 * M)
    acc[...] = jnp.zeros_like(acc)
    xT_v[M // 2:M // 2 + 8, :] = jnp.full((8, S), 0x3F803F80, U32)
    for r in range(NR):
        c0, c1 = r * RB, (r + 1) * RB
        c_x[r].wait()
        if r == 0:
            c_wq[0].start(); c_wq[1].start()
        if r == 2:
            c_c.start(); c_wuk[0].start(); c_wuk[1].start()
        xr = ld(xT_v, 0, M, c0, c1)
        t = _nn(wqkT, xr)
        p = phi(t[:2 * M]).astype(BF)
        g_s[:, c0:c1] = jax.nn.sigmoid(t[2 * M:2 * M + 8])
        st(pq_s, 0, M, p[:M], c0, c1)
        st(pk_s, 0, M, p[M:], c0, c1)
        st(x_s, c0, c1, xr.astype(F32).T.astype(BF))
    c_wuv[0].start(); c_wuv[1].start(); c_wo.start()
    NX("s2_gt")
    c_wob.wait()
    bst = {}
    def b_gt():
        bst["GT"] = _nt(ld(xT_v, 0, M + 16), ld(pk_s, 0, M))
    def b_kv():
        GT = bst["GT"]
        kvT = _tn(wv_b, GT[:M].astype(BF))
        ri = lax.broadcasted_iota(jnp.int32, (M, M), 0) // DH
        ci = lax.broadcasted_iota(jnp.int32, (M, M), 1) // DH
        bst["kvT"] = jnp.where(ri == ci, kvT, 0.0).astype(BF)
        z = GT[M:M + 1, :]
        rz = lax.broadcasted_iota(jnp.int32, (HB, M), 0)
        cz = lax.broadcasted_iota(jnp.int32, (HB, M), 1) // DH
        bst["ZcT"] = jnp.where(rz == cz, z, 0.0).astype(BF)
    def b_tt():
        bst["TT"] = _tn(ld(wob_v, 0, M), bst["kvT"]).astype(BF)

    def b_stage2(r):
        c0, c1 = r * RB, (r + 1) * RB
        pq = ld(pq_s, 0, M, c0, c1)
        den = _nn(bst["ZcT"], pq) + 1e-6
        rc = 1.0 / den
        sub = lax.broadcasted_iota(jnp.int32, (8, RB), 0)
        parts = []
        for v_ in range(M // 8):
            h0 = (8 * v_) // DH
            lo_ = jnp.broadcast_to(rc[h0:h0 + 1, :], (8, RB))
            nb = (h0 + 1) * DH - 8 * v_
            if nb < 8:
                lo_ = jnp.where(sub < nb, lo_, jnp.broadcast_to(rc[h0 + 1:h0 + 2, :], (8, RB)))
            parts.append(lo_)
        rf = jnp.concatenate(parts, axis=0)
        o = (pq.astype(F32) * rf).astype(BF)
        b_s[:, c0:c1] = _nn(bst["TT"], o)

    NQ = S // BQ
    nsub = BQ // T128

    def extract_one(refs, rows, dst, h):
        hv = _extract(refs, rows, h)
        for half in range(2):
            st(dst, 0, rows, hv[half], half * 128, half * 128 + 128)

    def extract(h):
        extract_one((wuk_v0, wuk_v1), DC, wuk_s, h)
        extract_one((wuv_v0, wuv_v1), DC, wuv_s, h)

    def extract_q_all():
        for j in range(H // 2):
            for half, w in enumerate((wq_v0, wq_v1)):
                a = w[pl.ds(j, M, stride=8), :]
                cols = slice(half * 128, half * 128 + 128)
                wq_s[2 * j, :, cols] = pltpu.bitcast(a.astype(jnp.uint16), U32)
                wq_s[2 * j + 1, :, cols] = pltpu.bitcast((a >> 16).astype(jnp.uint16), U32)

    def q_head(h, carry):
        w = pltpu.bitcast(wq_s[h], BF)
        for r in range(S // PB):
            r0, r1 = r * PB, (r + 1) * PB
            q = (_nn(ld(x_s, r0, r1), w) * (LOG2E / 16.0)).astype(BF)
            q_s[h, r0 // 2:r1 // 2, :] = pltpu.bitcast(q, U32)
        return carry
    def proj_k(r0, r1):
        st(k_s, r0, r1, _nn(ld(c_v, r0, r1), ld(wuk_s, 0, DC)).astype(BF))
    def proj_v(r0, r1):
        st(v_s, r0, r1, _nn(ld(c_v, r0, r1), ld(wuv_s, 0, DC)).astype(BF))
    def proj():
        for r in range(S // PB):
            r0, r1 = r * PB, (r + 1) * PB
            proj_k(r0, r1); proj_v(r0, r1)

    def qk(h, i):
        r0 = i * BQ
        a = lax.broadcasted_iota(jnp.int32, (T128, T128), 0)
        b = lax.broadcasted_iota(jnp.int32, (T128, T128), 1)
        s_diag = []
        q = pltpu.bitcast(q_s[h, r0 // 2:(r0 + BQ) // 2, :], BF)
        for t in range(nsub):
            s = _nt(q[t * T128:(t + 1) * T128, :], ld(k_s, r0, r0 + (t + 1) * T128))
            last = jnp.where(b <= a, s[:, t * T128:], NEG)
            s_diag.append(jnp.concatenate([s[:, :t * T128], last], axis=1) if t > 0 else last)
        m = jnp.concatenate([jnp.max(s, axis=-1, keepdims=True) for s in s_diag], axis=0)
        s_off = None
        if i > 0:
            s_off = _nt(q, ld(k_s, 0, r0))
            m = jnp.maximum(jnp.max(s_off, axis=-1, keepdims=True), m)
        return s_diag, s_off, m

    def pv(i, state):
        s_diag, s_off, m = state
        r0 = i * BQ
        cs, ls = [], []
        for t in range(nsub):
            p = jnp.exp2(s_diag[t] - m[t * T128:(t + 1) * T128, :])
            ls.append(jnp.sum(p, axis=1, keepdims=True))
            cs.append(_nn(p.astype(BF), ld(v_s, r0, r0 + (t + 1) * T128)))
        l = jnp.concatenate(ls, axis=0)
        ctx = jnp.concatenate(cs, axis=0)
        if i > 0:
            KC = PVC if PVC else r0
            for k0 in range(0, r0, KC):
                k1 = min(r0, k0 + KC)
                p_off = jnp.exp2(s_off[:, k0:k1] - m)
                l = l + jnp.sum(p_off, axis=1, keepdims=True)
                ctx = ctx + _nn(p_off.astype(BF), ld(v_s, k0, k1))
        if RCP:
            return (ctx * (1.0 / l)).astype(BF)
        return (ctx / l).astype(BF)

    def out_copy(i):
        r0 = i * BQ
        return pltpu.make_async_copy(o_s.bitcast(BF).at[:, r0:r0 + BQ], o_hbm.at[:, r0:r0 + BQ], osems.at[i])

    def oproj(i, cn, woT_h, final):
        r0 = i * BQ
        a = acc[:, r0:r0 + BQ] + _nt(woT_h, cn)
        if not final:
            acc[:, r0:r0 + BQ] = a
        else:
            g = g_s[0:1, r0:r0 + BQ]
            st(o_s, 0, M, (g * a + (1.0 - g) * b_s[:, r0:r0 + BQ]).astype(BF), r0, r0 + BQ)
            out_copy(i).start()

    def attention(h, final):
        woT_h = pltpu.bitcast(woT_v[pl.ds(pl.multiple_of(h * (M // 2), M // 2), M // 2), :], BF)
        order = list(range(NQ))[::-1] if ORD == 0 else (list(range(NQ)) if ORD == 1 else [0] + list(range(NQ))[:0:-1])
        st_ = qk(h, order[0])
        prev = None
        for n, i in enumerate(order):
            nxt = qk(h, order[n + 1]) if n + 1 < NQ else None
            cn = pv(i, st_)
            if prev is not None:
                oproj(order[n - 1], prev, woT_h, final)
            prev = cn
            st_ = nxt
            if n == max(EXT_AT, 0) and EXT_AT != -1 and not final:
                extract(h + 1)
        oproj(order[-1], prev, woT_h, final)

    zero = jnp.int32(0)
    NX("s3_wqwait")
    c_wq[0].wait(); c_wq[1].wait()
    NX("s4_b2")
    extract_q_all()
    fill = {0: b_gt, 2: b_kv, 4: b_tt, 6: lambda: b_stage2(0), 8: lambda: b_stage2(1),
            10: lambda: b_stage2(2), 12: lambda: b_stage2(3)}
    if QUN:
        for h in range(H):
            if h in fill:
                fill[h]()
            q_head(h, 0)
    else:
        for k_ in sorted(fill):
            fill[k_]()
        NX("s5_qloop")
        lax.fori_loop(0, H, q_head, 0)
    NX("s6_wait")
    c_c.wait(); c_wuk[0].wait(); c_wuk[1].wait()
    c_wuv[0].wait(); c_wuv[1].wait(); c_wo.wait()
    NX("s7_proj0")
    extract(zero)
    proj()
    NX("s8_main")

    def head(h, carry):
        if SCOPES == 2:
            with jax.named_scope("l_att"):
                attention(h, False)
            with jax.named_scope("l_proj"):
                proj()
        else:
            attention(h, False)
            proj()
        return carry
    if UNROLL == 15:
        for h in range(H - 1):
            if SCOPES == 3:
                with jax.named_scope("head"):
                    head(jnp.int32(h), 0)
            else:
                head(jnp.int32(h), 0)
    else:
        def heads(it, carry):
            for j in range(UNROLL):
                head(it * UNROLL + j if EXT_AT != -2 else jnp.int32(3), 0)
            return carry
        lax.fori_loop(0, (H - 1) // UNROLL, heads, 0)
    NX("s9_last")
    attention(jnp.int32(H - 1), True)
    NX("s10_outwait")
    for i in range(NQ):
        out_copy(i).wait()
    NX(None)

def make(BQ=256, PB=512, RB=512, EXT_AT=0, SCOPES=False, UNROLL=1, QUN=True, PVC=0, RCP=False, ORD=0):
    def fn(A_x, A_c_kv, A_w_q, A_w_uk, A_w_uv, A_w_o, B_x, B_wqkv, B_wo, gate_w):
        ins = [A_x.transpose(0, 2, 1).reshape(M, S), A_c_kv.reshape(S, DC), A_w_q.reshape(M * H, D),
               A_w_uk.reshape(DC * H, D), A_w_uv.reshape(DC * H, D),
               A_w_o.transpose(0, 2, 1).reshape(H * M, D), B_wqkv, B_wo,
               gate_w]
        V = pltpu.VMEM
        scratch = [V((M // 2 + 8, S), U32), V((S // 2, DC), U32),
                   V((M * 8, 128), U32), V((M * 8, 128), U32), V((DC * 8, 128), U32), V((DC * 8, 128), U32),
                   V((DC * 8, 128), U32), V((DC * 8, 128), U32),
                   V((H * M // 2, D), U32), V((M // 2, 3 * M), U32), V((M // 2, M), U32), V((M,), BF)]
        qkv = [V((H, S // 2, D), U32), V((S // 2, D), U32), V((S // 2, D), U32),
               V((H, M // 2, D), U32), V((DC // 2, D), U32), V((DC // 2, D), U32)]
        scratch += [pltpu.SemaphoreType.DMA((15,)), pltpu.SemaphoreType.DMA((S // BQ,)),
                    V((M, S), F32), V((M, S), F32), V((8, S), F32),
                    *qkv,
                    V((M // 2, S), U32), V((M // 2, S), U32), V((S // 2, M), U32), V((M // 2, S), U32)]
        def kern(*refs):
            return kernel(*refs, BQ=BQ, PB=PB, RB=RB, EXT_AT=EXT_AT, SCOPES=SCOPES, UNROLL=UNROLL, QUN=QUN, PVC=PVC, RCP=RCP, ORD=ORD)
        out = pl.pallas_call(
            kern,
            out_shape=jax.ShapeDtypeStruct((M, S), BF),
            in_specs=[pl.BlockSpec(memory_space=pltpu.HBM)] * 9,
            out_specs=pl.BlockSpec(memory_space=pltpu.HBM),
            scratch_shapes=scratch,
            compiler_params=pltpu.CompilerParams(vmem_limit_bytes=110 * 1024 * 1024),
        )(*ins)
        return out.reshape(1, M, S).transpose(0, 2, 1)
    return fn


_impl = make(UNROLL=15, PVC=512)


@jax.jit
def pallas_gated_mix__compressed_kv_cla__linear_attn_block__prompt_kernel(
    A_x, A_c_kv, A_w_q, A_w_uk, A_w_uv, A_w_o, B_x, B_wqkv, B_wo, gate_w,
):
    return _impl(A_x, A_c_kv, A_w_q, A_w_uk, A_w_uv, A_w_o, B_x, B_wqkv, B_wo, gate_w)
```
